```python
import os as _os
_os.environ.setdefault("JAX_PLATFORMS", "cpu")
import jax
import jax.numpy as jnp

def _softmax(x, axis=-1):
    return jax.nn.softmax(x, axis=axis)
def _gelu(x):
    return jax.nn.gelu(x, approximate=True)
def _silu(x):
    return jax.nn.silu(x)
def _sigmoid(x):
    return jax.nn.sigmoid(x)
def _layernorm(x, axis=-1, eps=1e-5):
    m = jnp.mean(x, axis=axis, keepdims=True)
    v = jnp.var(x, axis=axis, keepdims=True)
    return (x - m) / jnp.sqrt(v + eps)
def _scatter_add(tgt, idx, src, axis=0):
    return tgt.at[idx].add(src)
def _segment_sum(src, seg, n):
    return jax.ops.segment_sum(src, seg, n)
class _Rng:
    def __init__(self, key):
        self._k = key
    def _next(self):
        self._k, sub = jax.random.split(self._k)
        return sub
    def normal(self, shape):
        return jax.random.normal(self._next(), shape, dtype=jnp.bfloat16)
    def randint(self, lo, hi, shape):
        return jax.random.randint(self._next(), shape, lo, hi, dtype=jnp.int32)
    def uniform(self, shape, lo=0.0, hi=1.0):
        return jax.random.uniform(self._next(), shape, jnp.bfloat16, lo, hi)
    def permutation(self, n):
        return jax.random.permutation(self._next(), n)


kernel_name = 'sequential_preLN__sliding_block__dense_activation_gelu__prompt'

def setup_inputs():
    _rng = _Rng(jax.random.key(int.from_bytes(__import__("os").urandom(4), "little")))
    _w = (lambda a: (lambda t: t.astype(jnp.bfloat16) if jnp.issubdtype(t.dtype, jnp.floating) else t)(jnp.asarray(a)))
    def _A_setup():
        B, S, D = 1, 2048, 640
        return {
            "x": _w((lambda *s: _rng.normal(s) * 0.05)(B, S, D)),
            "wqkv": _w((lambda *s: _rng.normal(s) * 0.05)(D, 3 * D)),
            "wo": _w((lambda *s: _rng.normal(s) * 0.05)(D, D)),
        }
    _A_in = _A_setup()

    def _B_setup():
        B, S, D, F = 1, 2048, 640, 1536
        return {
            "x": _w((lambda *s: _rng.normal(s) * 0.05)(B, S, D)),
            "w1": _w((lambda *s: _rng.normal(s) * 0.8)(D, F) * (D ** -0.5)),
            "b1": _w((lambda *s: _rng.normal(s) * 0.8)(F) * 0.01),
            "w2": _w((lambda *s: _rng.normal(s) * 0.8)(F, D) * (F ** -0.5)),
            "b2": _w((lambda *s: _rng.normal(s) * 0.05)(D) * 0.01),
        }
    _B_in = _B_setup()

    return {
        "A_x": _A_in["x"],
        "A_wqkv": _A_in["wqkv"],
        "A_wo": _A_in["wo"],
        "B_x": _B_in["x"],
        "B_w1": _B_in["w1"],
        "B_b1": _B_in["b1"],
        "B_w2": _B_in["w2"],
        "B_b2": _B_in["b2"],
    }

def reference(A_x, A_wqkv, A_wo, B_x, B_w1, B_b1, B_w2, B_b2):
    def _A_ref(x, wqkv, wo):
        B, S, D = x.shape
        H = 32; Dh = D // H; W = 256
        qkv = (lambda x, *d: x.transpose(*d))((x @ wqkv).reshape(B, S, 3, H, Dh), 2, 0, 3, 1, 4)
        q, k, v = qkv[0], qkv[1], qkv[2]
        scores = jnp.einsum("bhqd,bhkd->bhqk", q, k) * (Dh ** -0.5)
        idx = jnp.arange(S)
        mask = (idx[:, None] - idx[None, :] >= 0) & (idx[:, None] - idx[None, :] < W)
        scores = jnp.where(mask[None, None], scores, -1e9)
        p = _softmax(scores, axis=-1)
        o = jnp.einsum("bhqk,bhkd->bhqd", p, v)
        return (lambda x, *d: x.transpose(*d))(o, 0, 2, 1, 3).reshape(B, S, D) @ wo

    def _B_ref(x, w1, b1, w2, b2):
        h = jnp.einsum("bsd,df->bsf", x, w1) + b1
        h = _gelu(h)
        return jnp.einsum("bsf,fd->bsd", h, w2) + b2

    x = A_x
    h = x + _A_ref(_layernorm(x, axis=-1), A_wqkv, A_wo)
    h2 = h + _B_ref(_layernorm(h, axis=-1), B_w1, B_b1, B_w2, B_b2)
    return h2
```

```python
import functools
import math

import jax
import jax.numpy as jnp
import jax.experimental.pallas as pl
import jax.experimental.pallas.tpu as pltpu

T = 128
H = 32
DH = 20
G = 2
L1, L2, L3 = 3, 2, 2
LAG = 2
SPAN = 0.92
DLY = 2
SK0, SK1, PK0 = 0.76, 1.0, 0.8
NEG = -1e30
EPS = 1e-5
WI32 = True
f32, bf16, i32 = jnp.float32, jnp.bfloat16, jnp.int32


def _ln(x):
    m = jnp.mean(x, axis=-1, keepdims=True)
    c = x - m
    v = jnp.mean(c * c, axis=-1, keepdims=True)
    return c * jax.lax.rsqrt(v + EPS)


def _gelu(x):
    c = math.sqrt(2.0 / math.pi)
    hx = 0.5 * x
    return hx + hx * jnp.tanh(x * (c + (c * 0.044715) * (x * x)))


def _iota(shape, axis):
    return jax.lax.broadcasted_iota(i32, shape, axis)


def _rows(start, size, align):
    if not isinstance(start, int):
        start = pl.multiple_of(start, align)
    return pl.ds(start, size)


def _pack(x):
    return pltpu.bitcast(x.astype(bf16), i32)


def _bf(x):
    return pltpu.bitcast(x, bf16)


def _dot(a, b):
    return jnp.dot(a, b, preferred_element_type=f32)


def _kernel(x_hbm, wqkv_hbm, wo_hbm, w1_hbm, b1_ref, w2_hbm, b2_ref, out_hbm,
            x_s, wqkv, wo, w1, w2, out_s, kf_s, h_s, qt_s, vt_s, kr_s, kp_s,
            ot_s, o_s, bias_s, sems, osems, *, S, D, F):
    nb, nt, nf = S // T, D // T, F // T
    w = T // G
    hp = w // DH
    na = pl.cdiv(H, hp)
    nq, no = qt_s.shape[0], o_s.shape[0]
    col = lambda n: slice(n * T, (n + 1) * T)
    T2, w2_ = T // 2, w // 2
    wt = (lambda ref, n: _bf(ref[:, col(n)])) if WI32 else (lambda ref, n: ref[:, col(n)])
    wv_ = (lambda ref: ref.bitcast(bf16)) if WI32 else (lambda ref: ref)

    def stage_a(b, waits=None):
        val = {}

        def ln1():
            val['xn'] = _ln(x_s[_rows(b * T, T, T), :].astype(f32)).astype(bf16)

        def proj(kind, n):
            def run():
                if waits and (kind, n) in waits:
                    waits[kind, n]()
                kf_s[kind * nt + n] = _dot(val['xn'], wt(wqkv, kind * nt + n))
            return run

        def post(kind, n):
            def run():
                r = kf_s.at[kind * nt + n]
                if kind == 0:
                    val[0, n] = _pack((r[...] * (DH ** -0.5 * math.log2(math.e))).T)
                elif kind == 2:
                    val[2, n] = _pack(r[...].T)
                else:
                    k32 = _pack(jnp.concatenate([r[pl.ds(m + e, 8, stride=2), :]
                                                 for m in range(0, T, 16) for e in (0, 1)], axis=0))
                    for g in range(G):
                        kr_s[g, _rows(b * T2 + T2, T2, T2), col(n)] = pltpu.roll(k32, g * w, 1) if g else k32
            return run

        def skew(a):
            def run():
                c0, c1 = a * hp * DH, min((a + 1) * hp, H) * DH
                lane = _iota((T // 2, T), 1)
                acc = None
                for g in range(G):
                    for n in range(c0 // T, (c1 - 1) // T + 1):
                        lo, up = max(c0, n * T), min(c1, (n + 1) * T)
                        src = kr_s[g, _rows(b * T2 + (g + 1) * w2_, T2, w2_), col(n)]
                        if acc is None:
                            acc = src
                        else:
                            acc = jnp.where(((lane - (lo + g * w)) & (T - 1)) < up - lo, src, acc)
                kp_s[a, _rows(b * T2 + T, T2, T2), :] = acc
            return run

        order = [(kind, n) for kind in (1, 0, 2) for n in range(nt)]
        seq = []
        for j in range(len(order) + DLY):
            if j < len(order):
                seq.append((5, proj(*order[j])))
            if j >= DLY:
                seq.append((0, post(*order[j - DLY])))
        def commit(kind):
            def run():
                for n in range(nt):
                    (vt_s if kind else qt_s)[b if kind else b % nq, n * T2:(n + 1) * T2, :] = val[kind, n]
            return run

        return (0, ln1), seq, [skew(a) for a in range(na)], [commit(0), commit(2)]

    def stage_att(b):
        edge = b if isinstance(b, int) and b < 2 else None
        nblk = 2 * G + 1
        t0 = 0 if edge is None else (2 - edge) * G - (G - 1)
        ot = [None] * (D // 8)
        st, rs = {}, {}

        def key_row(n):
            r = _iota((n, T), 0)
            return (r & -16) + 2 * (r & 7) + ((r >> 3) & 1)

        def qk(h):
            lo = h * DH
            a0 = lo // 16 * 16
            r = _iota((16, T), 0)
            q32 = jnp.where((r >= (lo - a0) // 2) & (r < (lo - a0 + DH) // 2),
                            qt_s[b % nq, a0 // 2:a0 // 2 + 16, :], 0)
            parts = [jnp.zeros((8, T), i32)] * (T // 16)
            lane = _iota((8, T), 1)
            for g in range(G):
                for j in range(2):
                    v = q32[8 * j:8 * j + 8]
                    if G > 1:
                        v = jnp.where((lane >= g * w) & (lane < (g + 1) * w), v, 0)
                    parts[((a0 + g * w) // 16 + j) % (T // 16)] = v
            qh = pltpu.bitcast(jnp.concatenate(parts, axis=0), bf16)
            n = (nblk - t0) * w
            s = _dot(_bf(kp_s[h // hp, _rows(b * T2 + T2 + (t0 - 1) * w2_, n // 2, w2_), :]), qh)
            if edge is None:
                first = key_row(w) > (_iota((w, T), 1) & (w - 1))
                s = jnp.concatenate([jnp.where(first, s[:w], s[2 * T:]), s[w:2 * T]], axis=0)
            else:
                c = _iota((n, T), 1)
                key = key_row(n) + t0 * w + (c - (c & (w - 1))) - 2 * T
                s = jnp.where((key >= -T * edge) & (key <= c), s, NEG)
            st[h] = (s, jnp.max(s, axis=0, keepdims=True))

        def ex(h):
            s, m = st.pop(h)
            e = jnp.exp2(s - m)
            st[h] = jnp.concatenate(
                [pltpu.pack_elementwise([e[r:r + 8], e[r + 8:r + 16]], packed_dtype=bf16)
                 for r in range(0, s.shape[0], 16)], axis=0)

        def pv(h):
            n = 2 * T if edge is None else (nblk - t0) * w
            p32 = pltpu.bitcast(st.pop(h), i32)
            xs = [p32[j * w // 2:(j + 1) * w // 2] for j in range(n // w)]
            if edge is None:
                r2, c = 2 * _iota((w // 2, T), 0), _iota((w // 2, T), 1) & (w - 1)
                fm = jnp.where(r2 > c, 0xFFFF, 0) | jnp.where(r2 + 1 > c, -0x10000, 0)
                head = xs[0] & fm
                xs = [head] + xs[1:] + [xs[0] ^ head]
            else:
                xs = [None] * t0 + xs
            lane = _iota((w // 2, T), 1)
            d = 1
            while d < G:
                up = (lane & (d * w)) != 0
                get = lambda j: xs[j] if 0 <= j < len(xs) else None
                nxt = []
                for j in range(len(xs) + d):
                    hi_, lo_ = get(j - d), get(j)
                    if hi_ is None and lo_ is None:
                        nxt.append(None)
                    else:
                        nxt.append(jnp.where(up, 0 if hi_ is None else hi_, 0 if lo_ is None else lo_))
                xs, d = nxt, 2 * d
            j0 = 0 if edge is None else 2 - edge
            p = pltpu.bitcast(jnp.concatenate(xs[j0 * G:], axis=0), bf16)
            a0 = h * DH // 16 * 16
            r = _iota((16, T), 0)
            ones = (r >= 12) if h * DH - a0 <= 4 else (r < 4)
            vw = [_bf(jnp.where(ones, 0x3F803F80, vt_s[b - 2 + j, a0 // 2:a0 // 2 + 16, :]))
                  for j in range(j0, 3)]
            rs[h] = _dot(jnp.concatenate(vw, axis=1), p)

        def fin(h):
            r = rs.pop(h)
            lo, up = h * DH, (h + 1) * DH
            a0 = lo // 16 * 16
            li = 3 if lo - a0 <= 4 else 0
            inv = pl.reciprocal(r[li * 8:(li + 1) * 8], approx=False)
            for j in range(4):
                g0 = a0 + 8 * j
                if g0 + 8 <= lo or g0 >= up:
                    continue
                val = r[8 * j:8 * j + 8] * inv
                if ot[g0 // 8] is not None:
                    val = jnp.where(_iota((8, T), 0) >= lo - g0, val, ot[g0 // 8])
                ot[g0 // 8] = val
            if up // T > lo // T:
                n = lo // T
                ot_s[n] = jnp.concatenate(ot[n * T // 8:(n + 1) * T // 8], axis=0)

        def tr(h):
            n = h * DH // T
            if (h + 1) * DH // T > n:
                o_s[b % no, :, col(n)] = ot_s[n].T

        def slot(t):
            def run():
                for fn, lag in ((qk, 0), (ex, L1), (pv, L1 + L2), (fin, L1 + L2 + L3), (tr, L1 + L2 + L3 + 1)):
                    if 0 <= t - lag < H:
                        fn(t - lag)
            return run

        return [slot(t) for t in range(H + L1 + L2 + L3 + 1)]

    def stage_b(b, u=0):
        val = {}

        def oproj(n):
            def run():
                if n == 0:
                    val['o'] = o_s[b % no].astype(bf16)
                h_s[u, :, col(n)] = (x_s[_rows(b * T, T, T), col(n)].astype(f32)
                                     + _dot(val['o'], wt(wo, n)))
            return run

        def ln2():
            val['hn'] = _ln(h_s[u]).astype(bf16)

        def up(n):
            def run():
                a = _dot(val['hn'], wt(w1, n)) + bias_s[0:1, col(n)]
                val[n] = _gelu(a).astype(bf16)
            return run

        def down(n):
            def run():
                y = _dot(jnp.concatenate([val[m] for m in range(nf)], axis=1), wt(w2, n)) + bias_s[1:2, col(n)]
                out_s[_rows(b * T, T, T), col(n)] = (h_s[u, :, col(n)] + y).astype(out_s.dtype)
            return run

        return ([(5, oproj(n)) for n in range(nt)] + [(0, ln2)],
                [(5, up(n)) for n in range(nf)] + [(12, down(n)) for n in range(nt)])

    def emit(dense, *streams):
        total = sum(c for c, _ in dense)
        done, pos = 0, [0] * len(streams)
        for c, fn in dense + [(None, None)]:
            for k, (fns, lo, hi) in enumerate(streams if c != 0 else ()):
                while pos[k] < len(fns) and (c is None or (lo + (hi - lo) * pos[k] / len(fns)) * total <= done):
                    fns[pos[k]]()
                    pos[k] += 1
            if fn is not None:
                fn()
                done += c

    def out_copy(b):
        rows = _rows(b * T, T, T)
        return pltpu.make_async_copy(out_s.at[rows], out_hbm.at[rows], osems.at[b])

    def part(src, dst, idx, k):
        return pltpu.make_async_copy(src.at[idx], dst.at[idx], sems.at[k])

    x_a, x_b, x_c = (part(x_hbm, x_s, slice(lo * T, up * T), k)
                     for k, (lo, up) in enumerate(((0, 1), (1, 6), (6, nb))))
    wk, wq, wv = (part(wqkv_hbm, wv_(wqkv), (slice(None), slice(kind * D, (kind + 1) * D)), 3 + kind)
                  for kind in (1, 0, 2))
    ws = [pltpu.make_async_copy(s, wv_(d), sems.at[6 + k])
          for k, (s, d) in enumerate(((wo_hbm, wo), (w1_hbm, w1), (w2_hbm, w2)))]
    for c in (x_a, wk, wq, wv):
        c.start()
    for g in range(G):
        kr_s[g, 0:T2, :] = jnp.zeros((T2, D), i32)
    bias_s[0:1, :] = b1_ref[...].astype(f32).reshape(1, F)
    bias_s[1:2, 0:D] = b2_ref[...].astype(f32).reshape(1, D)
    x_a.wait()

    def after(c, *nxt):
        def run():
            c.wait()
            for n in nxt:
                n.start()
        return run

    ln1, seq, sk, cm = stage_a(0, {(1, 0): after(wk, x_b), (0, 0): after(wq, ws[0], ws[1]), (2, 0): after(wv, ws[2])})
    ln1[1]()
    nxt = stage_a(1)
    emit(seq[:8] + [(0, x_b.wait), nxt[0]] + seq[8:], (sk, PK0, 1.0), (cm, 1.0, 1.0))
    for j in range(LAG):
        _, seq, sk, cm = nxt
        nxt = stage_a(j + 2)
        emit(seq[:8] + [nxt[0]] * (j + 1 < LAG) + seq[8:], (stage_att(j), 0.0, 1.0), (sk, PK0, 1.0), (cm, 1.0, 1.0))
    for c in ws:
        c.wait()
    x_c.start()

    def body(j, carry):
        @pl.when(j == 5)
        def _():
            x_c.wait()
        b1, b2 = stage_b(j - LAG)
        ln1, seq, sk, cm = stage_a(j + 1)
        emit(b1[:1] + [ln1] + b1[1:] + seq + b2, (stage_att(j), 0.0, SPAN), (sk, SK0, SK1), (cm, 1.0, 1.0))
        out_copy(j - LAG).start()
        return carry

    jax.lax.fori_loop(LAG, nb - 1, body, 0)
    tail = [stage_b(b, b % 2) for b in range(nb - 1 - LAG, nb)]
    seq = tail[0][0]
    for k in range(len(tail) - 2):
        seq = seq + tail[k + 1][0] + tail[k][1] + [(0, out_copy(nb - 1 - LAG + k).start)]
    emit(seq, (stage_att(nb - 1), 0.0, SPAN))
    emit(tail[-1][0] + tail[-2][1] + [(0, out_copy(nb - 2).start)] + tail[-1][1])
    out_copy(nb - 1).start()
    for b in range(nb):
        out_copy(b).wait()


@jax.jit
def pallas_sequential_preLN__sliding_block__dense_activation_gelu__prompt_kernel(
    A_x: jax.Array,
    A_wqkv: jax.Array,
    A_wo: jax.Array,
    B_x: jax.Array,
    B_w1: jax.Array,
    B_b1: jax.Array,
    B_w2: jax.Array,
    B_b2: jax.Array,
):
    del B_x
    B, S, D = A_x.shape
    F = B_w1.shape[1]
    assert B == 1 and D == H * DH
    nb = S // T
    hbm = pl.BlockSpec(memory_space=pl.ANY)
    vmem = pl.BlockSpec(memory_space=pltpu.VMEM)
    packed = lambda *s: pltpu.VMEM(s[:-2] + (s[-2] // 2, s[-1]), i32)
    wbuf = packed if WI32 else (lambda *s: pltpu.VMEM(s, bf16))
    out = pl.pallas_call(
        functools.partial(_kernel, S=S, D=D, F=F),
        in_specs=[hbm, hbm, hbm, hbm, vmem, hbm, vmem],
        out_specs=hbm,
        out_shape=jax.ShapeDtypeStruct((S, D), A_x.dtype),
        scratch_shapes=[
            pltpu.VMEM((S, D), bf16),
            wbuf(D, 3 * D), wbuf(D, D), wbuf(D, F), wbuf(F, D),
            pltpu.VMEM((S, D), A_x.dtype),
            pltpu.VMEM((3 * D // T, T, T), f32),
            pltpu.VMEM((2, T, D), f32),
            packed(2, D, T),
            packed(nb, D, T),
            packed(G, S + T, D),
            packed(pl.cdiv(H, T // G // DH), S + 2 * T, T),
            pltpu.VMEM((D // T, T, T), f32),
            pltpu.VMEM((4, T, D), f32),
            pltpu.VMEM((8, F), f32),
            pltpu.SemaphoreType.DMA((9,)),
            pltpu.SemaphoreType.DMA((nb,)),
        ],
        compiler_params=pltpu.CompilerParams(vmem_limit_bytes=100 * 1024 * 1024),
    )(A_x.reshape(S, D), A_wqkv, A_wo, B_w1, B_b1, B_w2, B_b2)
    return out.reshape(B, S, D)
```

```python
import functools
import math

import jax
import jax.numpy as jnp
import jax.experimental.pallas as pl
import jax.experimental.pallas.tpu as pltpu

T = 128
H = 32
DH = 20
G = 4
NEG = -1e30
EPS = 1e-5
STEPS = (0, 3, 1, 3, 2, 2, 1)
DLY = 2
DS = 3
KS = 2
f32, bf16, i32 = jnp.float32, jnp.bfloat16, jnp.int32


def _ln(x):
    m = jnp.mean(x, axis=-1, keepdims=True)
    c = x - m
    v = jnp.mean(c * c, axis=-1, keepdims=True)
    return c * jax.lax.rsqrt(v + EPS)


def _gelu(x):
    c = math.sqrt(2.0 / math.pi)
    hx = 0.5 * x
    return hx + hx * jnp.tanh(x * (c + (c * 0.044715) * (x * x)))


def _iota(shape, axis):
    return jax.lax.broadcasted_iota(i32, shape, axis)


def _rows(start, size, align):
    if not isinstance(start, int):
        start = pl.multiple_of(start, align)
    return pl.ds(start, size)


def _pack_t(x):
    return pltpu.bitcast(x.astype(bf16).T, i32)


def _pack2(lo, hi):
    lo, hi = (jax.lax.bitcast_convert_type(t, i32) for t in (lo, hi))
    return jax.lax.shift_right_logical(lo, 16) | (hi & -0x10000)


def _bf(x):
    return pltpu.bitcast(x, bf16)


def _dot(a, b):
    return jnp.dot(a, b, preferred_element_type=f32)


def _kernel(x_hbm, wqkv_hbm, wo_hbm, w1_hbm, b1_hbm, w2_hbm, b2_hbm, out_hbm,
            x_s, wqkv, wo, w1, w2, out_s, kf_s, h_s, qt_s, vt_s, k_s, kr_s, kp_s,
            ot_s, o_s, b1_s, b2_s, bias_s, sems, osems, *, S, D, F):
    nb, nt, nf = S // T, D // T, F // T
    w = T // G
    hp = w // DH
    nq, no = qt_s.shape[0], o_s.shape[0] // T
    col = lambda n: slice(n * T, (n + 1) * T)
    T2, w2_ = T // 2, w // 2

    def stage_a(b, par, waits=None, kinds=(1, 0, 2), m=1):
        val = {}

        def ln1():
            val['xn'] = _ln(x_s[_rows(b * T, m * T, T), :].astype(f32)).astype(bf16)

        def proj(kind, n):
            def run():
                r = _dot(val['xn'], wqkv[:, col(kind * nt + n)])
                if waits and (kind, n) in waits:
                    waits[kind, n]()
                for u in range(m):
                    kf_s[par + u, kind * nt + n, 0:T, :] = r[u * T:(u + 1) * T]
            return run

        def post(u, kind, n):
            def run():
                r = kf_s.at[par + u, kind * nt + n]
                if kind == 0:
                    val[u, 0, n] = _pack_t(r[0:T, :] * (DH ** -0.5 * math.log2(math.e)))
                elif kind == 2:
                    val[u, 2, n] = _pack_t(r[0:T, :])
                else:
                    rows = lambda i: r[pl.ds(i, 8, stride=4), :].astype(bf16).astype(f32)
                    val[u, 1, n] = jnp.concatenate([_pack2(rows(i + e), rows(i + e + 2))
                                                 for i in range(0, T, 32) for e in (0, 1)], axis=0)
            return run

        order = [(kind, n) for kind in kinds for n in range(nt)]
        seq = []
        for j in range(len(order) + DLY):
            if j < len(order):
                seq.append((5 * m, proj(*order[j])))
            if j >= DLY:
                seq += [(0, post(u, *order[j - DLY])) for u in range(m)]

        def commit():
            for u in range(m):
                for n in range(nt):
                    qt_s[(b + u) % nq, n * T2:(n + 1) * T2, :] = val[u, 0, n]
                    k_s[_rows((b + u + 1) * T2, T2, T2), col(n)] = val[u, 1, n]
                    vt_s[b + u, n * T2:(n + 1) * T2, :] = val[u, 2, n]

        return (0, ln1), seq, [commit]

    def att_stages(b, par):
        edge = b if isinstance(b, int) and b < 2 else None
        nblk = 2 * G + 1
        t0 = 0 if edge is None else (2 - edge) * G - (G - 1)
        ot = [None] * (D // 8)
        st, rs, ks = {}, {}, {}

        def key_row(n):
            r = _iota((n, T), 0)
            return (r & -32) + 2 * (r & 15) + ((r >> 4) & 1)

        def rot(h):
            n = ((h // hp + 1) * hp * DH - 1) // T
            if n < nt and (h == 0 or (h % hp == 0 and n > (h * DH - 1) // T)):
                for g in range(G):
                    k32 = k_s[_rows(b * T2 + (g + 1) * w2_, T2, w2_), col(n)]
                    kr_s[par, g, :, col(n)] = pltpu.roll(k32, g * w, 1) if g else k32

        def skew(h):
            if h % hp:
                return
            c0, c1 = h * DH, min(h + hp, H) * DH
            lane = _iota((T2, T), 1)
            acc = None
            for g in range(G):
                for n in range(c0 // T, (c1 - 1) // T + 1):
                    lo, up = max(c0, n * T), min(c1, (n + 1) * T)
                    src = kr_s[par, g, :, col(n)]
                    if acc is None:
                        acc = src
                    else:
                        acc = jnp.where(((lane - (lo + g * w)) & (T - 1)) < up - lo, src, acc)
            if not (isinstance(b, int) and b == nb - 1):
                kp_s[h // hp, _rows(b * T2, T2, T2), :] = acc
            ks[h // hp] = acc

        def qk(h):
            lo = h * DH
            a0 = lo // 16 * 16
            r = _iota((16, T), 0)
            q32 = jnp.where((r >= (lo - a0) // 2) & (r < (lo - a0 + DH) // 2),
                            qt_s[b % nq, a0 // 2:a0 // 2 + 16, :], 0)
            parts = [jnp.zeros((8, T), i32)] * (T // 16)
            lane = _iota((8, T), 1)
            for g in range(G):
                for j in range(2):
                    v = q32[8 * j:8 * j + 8]
                    if G > 1:
                        v = jnp.where((lane >= g * w) & (lane < (g + 1) * w), v, 0)
                    parts[((a0 + g * w) // 16 + j) % (T // 16)] = v
            qh = pltpu.bitcast(jnp.concatenate(parts, axis=0), bf16)
            n = (nblk - t0) * w
            kw = ks[h // hp]
            if n > T:
                kw = jnp.concatenate([kp_s[h // hp, _rows(b * T2 - (n - T) // 2, (n - T) // 2, w2_), :], kw], axis=0)
            s = _dot(_bf(kw), qh)
            if edge is None:
                first = key_row(w) > (_iota((w, T), 1) & (w - 1))
                s = jnp.concatenate([jnp.where(first, s[:w], s[2 * T:]), s[w:2 * T]], axis=0)
            else:
                c = _iota((n, T), 1)
                key = key_row(n) + t0 * w + (c - (c & (w - 1))) - 2 * T
                s = jnp.where((key >= -T * edge) & (key <= c), s, NEG)
            st[h] = (s, jnp.max(s, axis=0, keepdims=True))

        def ex(h):
            s, m = st.pop(h)
            e = jnp.exp2(s - m)
            st[h] = jnp.concatenate([_pack2(e[r:r + 16], e[r + 16:r + 32])
                                     for r in range(0, s.shape[0], 32)], axis=0)

        def pv(h):
            n = 2 * T if edge is None else (nblk - t0) * w
            p32 = st.pop(h)
            xs = [p32[j * w // 2:(j + 1) * w // 2] for j in range(n // w)]
            if edge is None:
                r2, c = 2 * _iota((w // 2, T), 0), _iota((w // 2, T), 1) & (w - 1)
                fm = jnp.where(r2 > c, 0xFFFF, 0) | jnp.where(r2 + 1 > c, -0x10000, 0)
                head = xs[0] & fm
                xs = [head] + xs[1:] + [xs[0] ^ head]
            else:
                xs = [None] * t0 + xs
            lane = _iota((w // 2, T), 1)
            d = 1
            while d < G:
                up = (lane & (d * w)) != 0
                get = lambda j: xs[j] if 0 <= j < len(xs) else None
                nxt = []
                for j in range(len(xs) + d):
                    hi_, lo_ = get(j - d), get(j)
                    if hi_ is None and lo_ is None:
                        nxt.append(None)
                    else:
                        nxt.append(jnp.where(up, 0 if hi_ is None else hi_, 0 if lo_ is None else lo_))
                xs, d = nxt, 2 * d
            j0 = 0 if edge is None else 2 - edge
            p = pltpu.bitcast(jnp.concatenate(xs[j0 * G:], axis=0), bf16)
            a0 = h * DH // 16 * 16
            r = _iota((16, T), 0)
            ones = (r >= 12) if h * DH - a0 <= 4 else (r < 4)
            vw = [_bf(jnp.where(ones, 0x3F803F80, vt_s[b - 2 + j, a0 // 2:a0 // 2 + 16, :]))
                  for j in range(j0, 3)]
            rs[h] = _dot(jnp.concatenate(vw, axis=1), p)

        def fin(h):
            r = rs.pop(h)
            lo, up = h * DH, (h + 1) * DH
            a0 = lo // 16 * 16
            li = 3 if lo - a0 <= 4 else 0
            inv = pl.reciprocal(r[li * 8:(li + 1) * 8], approx=False)
            for j in range(4):
                g0 = a0 + 8 * j
                if g0 + 8 <= lo or g0 >= up:
                    continue
                val = r[8 * j:8 * j + 8] * inv
                if ot[g0 // 8] is not None:
                    val = jnp.where(_iota((8, T), 0) >= lo - g0, val, ot[g0 // 8])
                ot[g0 // 8] = val
            if up // T > lo // T:
                n = lo // T
                ot_s[par, n] = jnp.concatenate(ot[n * T // 8:(n + 1) * T // 8], axis=0)

        def tr(h):
            n = h * DH // T
            if (h + 1) * DH // T > n:
                o_s[_rows(b % no * T, T, T), col(n)] = ot_s[par, n].T

        return rot, skew, qk, ex, pv, fin, tr

    def stage_att(*blocks):
        stages = [att_stages(b, k % 2) for k, b in enumerate(blocks)]
        lags = [sum(STEPS[:k + 1]) for k in range(len(STEPS))]
        n = H * len(blocks)

        def slot(t):
            def run():
                for k in reversed(range(len(lags))):
                    if 0 <= t - lags[k] < n:
                        stages[(t - lags[k]) // H][k]((t - lags[k]) % H)
            return run

        return [slot(t) for t in range(n + lags[-1])]

    def stage_b(b, u=0, m=1):
        val = {}
        hr, xr = slice(u * T, (u + m) * T), _rows(b * T, m * T, T)

        def oproj(n):
            def run():
                if n == 0:
                    val['o'] = o_s[_rows(b % no * T, m * T, T), :].astype(bf16)
                h_s[hr, col(n)] = (x_s[xr, col(n)].astype(f32)
                                     + _dot(val['o'], wo[:, col(n)]))
            return run

        def ln2():
            val['hn'] = _ln(h_s[hr, :]).astype(bf16)

        def up(n):
            def run():
                a = _dot(val['hn'], w1[:, col(n)]) + bias_s[0:1, col(n)]
                val[n] = _gelu(a).astype(bf16)
            return run

        def down(n, p):
            def run():
                k0, k1 = p * nf // DS, (p + 1) * nf // DS
                y = _dot(jnp.concatenate([val[m] for m in range(k0, k1)], axis=1),
                         w2[k0 * T:k1 * T, col(n)])
                y = y + (val['y'] if p else bias_s[1:2, col(n)])
                if p < DS - 1:
                    val['y'] = y
                    return
                out_s[xr, col(n)] = (h_s[hr, col(n)] + y).astype(out_s.dtype)
            return run

        return ([(5 * m, oproj(n)) for n in range(nt)] + [(0, ln2)],
                [(5 * m, up(n)) for n in range(nf)] + [(12 * m / DS, down(n, p)) for n in range(nt) for p in range(DS)])

    def emit(dense, *streams):
        total = sum(c for c, _ in dense)
        done, pos = 0, [0] * len(streams)
        for c, fn in dense + [(None, None)]:
            for k, (fns, lo, hi) in enumerate(streams if c != 0 else ()):
                while pos[k] < len(fns) and (c is None or (lo + (hi - lo) * pos[k] / len(fns)) * total <= done):
                    fns[pos[k]]()
                    pos[k] += 1
            if fn is not None:
                fn()
                done += c

    def out_copy(b):
        rows = _rows(b * T, T, T)
        return pltpu.make_async_copy(out_s.at[rows], out_hbm.at[rows], osems.at[b])

    def part(src, dst, idx, k):
        return pltpu.make_async_copy(src.at[idx], dst.at[idx], sems.at[k])

    x_a, x_b, x_c = (part(x_hbm, x_s, slice(lo * T, up * T), k)
                     for k, (lo, up) in enumerate(((0, 3), (3, 6), (6, nb))))
    wk0, wk1, wq, wv = (part(wqkv_hbm, wqkv, (slice(None), slice(lo * T, up * T)), 3 + k)
                        for k, (lo, up) in enumerate(((nt, nt + KS), (nt + KS, 2 * nt), (0, nt), (2 * nt, 3 * nt))))
    ws = [pltpu.make_async_copy(s, d, sems.at[7 + k]) for k, (s, d) in enumerate(
        ((wo_hbm, wo), (w1_hbm, w1), (w2_hbm, w2), (b1_hbm, b1_s), (b2_hbm, b2_s)))]

    ws, bs = ws[:3], ws[3:]

    def after(c, *nxt):
        def run():
            c.wait()
            for n in nxt:
                n.start()
        return run

    for c in (x_a, wk0):
        c.start()
    k_s[0:T2, :] = jnp.zeros((T2, D), i32)
    kf_s[:, nt:2 * nt, T:, :] = jnp.zeros((3, nt, 32, T), f32)
    after(x_a, wk1)()
    bwait = lambda: (bs[0].wait(), bs[1].wait(), x_b.wait(), after(wv, *ws[1:])())
    pro = [stage_a(0, 0), stage_a(1, 1),
           stage_a(2, 2, {(1, KS - 1): after(wk1, wv, x_b, *bs), (1, nt - 1): after(wq, ws[0]), (0, nt - 1): bwait}),
           stage_a(3, 0, kinds=(0, 2, 1))]
    for a in pro[:3]:
        a[0][1]()
    after(wk0, wq)()
    cut = 4 * nt
    emit([c for cs in zip(*(a[1][:cut] for a in pro[:3])) for c in cs])
    bias_s[0:1, 0:F] = b1_s[...].astype(f32).reshape(1, F)
    bias_s[1:2, 0:D] = b2_s[...].astype(f32).reshape(1, D)
    rest = lambda a: a[1][cut:] + [(0, a[2][0])]
    emit(rest(pro[0]) + [pro[3][0]] + rest(pro[1]) + rest(pro[2]) + pro[3][1] + [(0, pro[3][2][0])],
         (stage_att(0, 1), 0.14, 0.9))
    for c in ws:
        c.wait()
    x_c.start()

    def body(i, carry):
        j = 2 + 2 * i
        pl.when(i == 1)(x_c.wait)
        b1, b2 = stage_b(j - 2, m=2)
        ln1, seq, cm = stage_a(j + 2, 0, m=2)
        emit(b1[:3] + [ln1] + b1[3:] + seq + b2, (stage_att(j, j + 1), 0.0, 0.96), (cm, 1.0, 1.0))
        out_copy(j - 2).start()
        out_copy(j - 1).start()
        return carry

    jax.lax.fori_loop(0, (nb - 4) // 2, body, 0)

    tail = [stage_b(b, b % 2) for b in range(nb - 4, nb)]
    done = lambda k: tail[k][1] + [(0, out_copy(nb - 4 + k).start)]
    emit(tail[0][0] + tail[1][0] + done(0) + done(1), (stage_att(nb - 2, nb - 1), 0.0, 0.95))
    last = [pltpu.make_async_copy(out_s.at[S - T:, col(n)], out_hbm.at[S - T:, col(n)], osems.at[nb - 1 + n])
            for n in range(nt)]
    seq = tail[3][1][:nf]
    for n in range(nt):
        seq = seq + tail[3][1][nf + n * DS:nf + (n + 1) * DS] + [(0, last[n].start)]
    emit(tail[2][0] + tail[3][0] + done(2) + seq)
    for c in [out_copy(b) for b in range(nb - 1)] + last:
        c.wait()


@jax.jit
def pallas_sequential_preLN__sliding_block__dense_activation_gelu__prompt_kernel(
    A_x: jax.Array,
    A_wqkv: jax.Array,
    A_wo: jax.Array,
    B_x: jax.Array,
    B_w1: jax.Array,
    B_b1: jax.Array,
    B_w2: jax.Array,
    B_b2: jax.Array,
):
    del B_x
    B, S, D = A_x.shape
    F = B_w1.shape[1]
    assert B == 1 and D == H * DH and S % (2 * T) == 0 and S >= 8 * T
    nb = S // T
    hbm = pl.BlockSpec(memory_space=pl.ANY)
    packed = lambda *s: pltpu.VMEM(s[:-2] + (s[-2] // 2, s[-1]), i32)
    out = pl.pallas_call(
        functools.partial(_kernel, S=S, D=D, F=F),
        in_specs=[hbm] * 7,
        out_specs=hbm,
        out_shape=jax.ShapeDtypeStruct((S, D), A_x.dtype),
        scratch_shapes=[
            pltpu.VMEM((S, D), bf16),
            pltpu.VMEM((D, 3 * D), bf16),
            pltpu.VMEM((D, D), bf16),
            pltpu.VMEM((D, F), bf16),
            pltpu.VMEM((F, D), bf16),
            pltpu.VMEM((S, D), A_x.dtype),
            pltpu.VMEM((3, 3 * D // T, T + 32, T), f32),
            pltpu.VMEM((2 * T, D), f32),
            packed(4, D, T),
            packed(nb, D, T),
            packed(S + T, D),
            packed(2, G, T, D),
            packed(pl.cdiv(H, T // G // DH), S, T),
            pltpu.VMEM((2, D // T, T, T), f32),
            pltpu.VMEM((4 * T, D), f32),
            pltpu.VMEM((F,), B_b1.dtype), pltpu.VMEM((D,), B_b2.dtype),
            pltpu.VMEM((8, F), f32),
            pltpu.SemaphoreType.DMA((12,)),
            pltpu.SemaphoreType.DMA((nb - 1 + D // T,)),
        ],
        compiler_params=pltpu.CompilerParams(vmem_limit_bytes=100 * 1024 * 1024),
    )(A_x.reshape(S, D), A_wqkv, A_wo, B_w1, B_b1, B_w2, B_b2)
    return out.reshape(B, S, D)
```
